```python
import os as _os
_os.environ.setdefault("JAX_PLATFORMS", "cpu")
import jax
import jax.numpy as jnp

def _softmax(x, axis=-1):
    return jax.nn.softmax(x, axis=axis)
def _gelu(x):
    return jax.nn.gelu(x, approximate=True)
def _silu(x):
    return jax.nn.silu(x)
def _sigmoid(x):
    return jax.nn.sigmoid(x)
def _layernorm(x, axis=-1, eps=1e-5):
    m = jnp.mean(x, axis=axis, keepdims=True)
    v = jnp.var(x, axis=axis, keepdims=True)
    return (x - m) / jnp.sqrt(v + eps)
def _scatter_add(tgt, idx, src, axis=0):
    return tgt.at[idx].add(src)
def _segment_sum(src, seg, n):
    return jax.ops.segment_sum(src, seg, n)
class _Rng:
    def __init__(self, key):
        self._k = key
    def _next(self):
        self._k, sub = jax.random.split(self._k)
        return sub
    def normal(self, shape):
        return jax.random.normal(self._next(), shape, dtype=jnp.bfloat16)
    def randint(self, lo, hi, shape):
        return jax.random.randint(self._next(), shape, lo, hi, dtype=jnp.int32)
    def uniform(self, shape, lo=0.0, hi=1.0):
        return jax.random.uniform(self._next(), shape, jnp.bfloat16, lo, hi)
    def permutation(self, n):
        return jax.random.permutation(self._next(), n)


kernel_name = 'gated_mix__sliding_local_dilated__linear_attn_block__prompt'

def setup_inputs():
    _rng = _Rng(jax.random.key(int.from_bytes(__import__("os").urandom(4), "little")))
    _w = (lambda a: (lambda t: t.astype(jnp.bfloat16) if jnp.issubdtype(t.dtype, jnp.floating) else t)(jnp.asarray(a)))
    def _A_setup():
        B, S, D = 1, 2048, 448
        return {
            "x": _w((lambda *s: _rng.normal(s) * 0.05)(B, S, D)),
            "wqkv": _w((lambda *s: _rng.normal(s) * 0.8)(D, 3 * D)),
            "wo": _w((lambda *s: _rng.normal(s) * 0.05)(D, D)),
        }
    _A_in = _A_setup()

    def _B_setup():
        B, S, D = 1, 2048, 448
        return {
            "x": _w((lambda *s: _rng.normal(s) * 0.05)(B, S, D)),
            "wqkv": _w((lambda *s: _rng.normal(s) * 1.6)(D, 3 * D)),
            "wo": _w((lambda *s: _rng.normal(s) * 0.8)(D, D)),
        }
    _B_in = _B_setup()

    return {
        "A_x": _A_in["x"],
        "A_wqkv": _A_in["wqkv"],
        "A_wo": _A_in["wo"],
        "B_x": _B_in["x"],
        "B_wqkv": _B_in["wqkv"],
        "B_wo": _B_in["wo"],
        "gate_w": _w((lambda *s: _rng.normal(s) * 0.05)(448) * 16.0),
    }

def reference(A_x, A_wqkv, A_wo, B_x, B_wqkv, B_wo, gate_w):
    def _A_ref(x, wqkv, wo):
        B, S, D = x.shape
        H = 16; Dh = D // H
        W, dil = 8, 2
        qkv = (lambda x, *d: x.transpose(*d))((x @ wqkv).reshape(B, S, 3, H, Dh), 2, 0, 3, 1, 4)
        q, k, v = qkv[0], qkv[1], qkv[2]
        scale = Dh ** -0.5
        pos = jnp.arange(S)
        off = jnp.arange(W) * dil
        idx = pos[:, None] - off[None, :]
        mask = idx >= 0
        idx_c = jnp.where(mask, idx, 0).reshape(-1)
        kg = k[:, :, idx_c, :].reshape(B, H, S, W, Dh)
        vg = v[:, :, idx_c, :].reshape(B, H, S, W, Dh)
        logits = jnp.einsum("bhsd,bhswd->bhsw", q, kg) * scale
        logits = jnp.where(mask[None, None, :, :], logits, -1e9)
        attn = _softmax(logits, axis=-1)
        o = jnp.einsum("bhsw,bhswd->bhsd", attn, vg)
        return (lambda x, *d: x.transpose(*d))(o, 0, 2, 1, 3).reshape(B, S, D) @ wo

    def _B_ref(x, wqkv, wo):
        B, S, D = x.shape
        H = 16; Dh = D // H
        qkv = (lambda x, *d: x.transpose(*d))((x @ wqkv).reshape(B, S, 3, H, Dh), 2, 0, 3, 1, 4)
        q, k, v = qkv[0], qkv[1], qkv[2]
        phi = lambda t: jnp.where(t > 0, t + 1, jnp.exp(t)) + 1e-6
        pq, pk = phi(q), phi(k)
        kv = jnp.einsum("bhsd,bhse->bhde", pk, v)
        z = jnp.einsum("bhsd->bhd", pk)
        num = jnp.einsum("bhqd,bhde->bhqe", pq, kv)
        den = jnp.einsum("bhqd,bhd->bhq", pq, z)[..., None] + 1e-6
        o = num / den
        return (lambda x, *d: x.transpose(*d))(o, 0, 2, 1, 3).reshape(B, S, D) @ wo

    x = A_x
    g = _sigmoid((x * gate_w).sum(-1, keepdims=True))
    a = _A_ref(x, A_wqkv, A_wo)
    b = _B_ref(x, B_wqkv, B_wo)
    return g * a + (1 - g) * b
```

```python
import functools
import jax
import jax.numpy as jnp
from jax import lax
import jax.experimental.pallas as pl
import jax.experimental.pallas.tpu as pltpu

S = 2048
D = 448
H = 16
DH = 28
W = 8
L = 128
NB = S // L
KT = 4
GR = 4 * DH
F32 = jnp.float32
BF16 = jnp.bfloat16
U32 = jnp.uint32
NT = (((1,), (1,)), ((), ()))
XS = (0, 2, 6, NB)


def _ktile(kt):
    k0 = kt * L
    return k0, min(L, D - k0)


def _pk(v):
    return pltpu.bitcast(v, U32)


def _up(v):
    return pltpu.bitcast(v, BF16)


def _lhs(ref, r0=None, r1=None, ntiles=KT, last=64):
    rs = slice(None) if r0 is None else slice(r0 // 2, r1 // 2)
    parts = [_up(ref[t, rs, :]) for t in range(ntiles - 1)]
    parts.append(_up(ref[ntiles - 1, rs, 0:last]))
    return jnp.concatenate(parts, axis=1)


def _phi(t):
    return jnp.where(t > 0, t + 1.0, jnp.exp(t)) + 1e-6


def _recip(x):
    r = pl.reciprocal(x, approx=True)
    return r * (2.0 - x * r)


def _yrow_a(r):
    return (r // 16) * L + GR + r % 16 if r < 64 else D + r


def _yrow_b(r):
    return (r // GR) * L + r % GR


def _kernel(x_hbm, wa_hbm, woa_hbm, wb_hbm, wob_hbm, gw_hbm, o_hbm,
            x_ref, wa_ref, woa_ref, wb_ref, wob_ref, gw_ref, o_ref,
            t_ref, w1_ref, w2_ref, wo_ref, wvt_ref, pk_ref, g_ref, zb_ref,
            q_ref, k_ref, v_ref, oh_ref, y_ref, sems, osems):
    def cp(src, dst, n):
        return pltpu.make_async_copy(src, dst, sems.at[n])

    c_wbk = cp(wb_hbm.at[:, 384:896], wb_ref.at[:, 384:896], 0)
    c_x = [cp(x_hbm.at[:, XS[j] * L:XS[j + 1] * L], x_ref.at[:, XS[j] * L:XS[j + 1] * L], 1 + j)
           for j in range(3)]
    c_w = [cp(wa_hbm, wa_ref, 4),
           cp(wb_hbm.at[:, 0:384], wb_ref.at[:, 0:384], 5),
           cp(gw_hbm, gw_ref, 6),
           cp(wb_hbm.at[:, 896:3 * D], wb_ref.at[:, 896:3 * D], 7),
           cp(woa_hbm, woa_ref, 8),
           cp(wob_hbm, wob_ref, 9)]
    for c in [c_wbk] + c_x + c_w:
        c.start()

    A0, QB0 = 16, 16 + 3 * D

    def prep1():
        for kt in range(KT):
            k0, kn = _ktile(kt)
            bt = wb_ref[k0:k0 + kn, 384:896].T
            w1_ref[kt, :, 0:kn] = _pk(bt[64:512])

    def prep2():
        gw = gw_ref[...].reshape(1, D)
        for kt in range(KT):
            k0, kn = _ktile(kt)
            w2_ref[kt, 0:8, 0:kn] = _pk(jnp.broadcast_to(gw[:, k0:k0 + kn], (16, kn)))
            t_ref[kt, 0:3 * D, 0:kn] = wa_ref[k0:k0 + kn, :].T.astype(F32)
        for t in range(3):
            for d in range(DH):
                for kt in range(KT):
                    k0, kn = _ktile(kt)
                    rows = t_ref[kt, pl.ds(D * t + d, H, stride=DH), :]
                    r0 = (A0 + D * t + H * d) // 2
                    w2_ref[kt, r0:r0 + 8, 0:kn] = _pk(rows[:, 0:kn].astype(BF16))
        for kt in range(KT):
            k0, kn = _ktile(kt)
            bt = wb_ref[k0:k0 + kn, 0:512].T
            w2_ref[kt, QB0 // 2:(QB0 + D) // 2, 0:kn] = _pk(bt[0:D])
            wvt_ref[kt, :, 0:kn] = _pk(wb_ref[k0:k0 + kn, 2 * D:3 * D].T)
        for nt in range(KT):
            n0, nn = _ktile(nt)
            t_ref[nt, 3 * D:4 * D, 0:nn] = woa_ref[:, n0:n0 + nn].astype(F32)
        for nt in range(KT):
            n0, nn = _ktile(nt)
            pa = [t_ref[nt, pl.ds(3 * D + d, H, stride=DH), :][:, 0:nn].astype(BF16)
                  for d in range(DH)]
            rows = []
            for j in range(4):
                rows += [wob_ref[GR * j:GR * (j + 1), n0:n0 + nn], pa[j]]
            pt = jnp.concatenate(rows + pa[4:], axis=0).T
            for j in range(7):
                wo_ref[j, n0 // 2:(n0 + nn) // 2, :] = _pk(pt[:, j * L:(j + 1) * L])

    ones = jnp.ones((64, 4 * L), BF16)

    def p1_proj(i):
        kb = jnp.dot(_lhs(w1_ref), x_ref[:, i * L:(i + 1) * L], preferred_element_type=F32)
        pk_ref[i] = _pk(_phi(kb).astype(BF16))

    def p1_g(c):
        for nt in range(KT):
            n0, nn = _ktile(nt)
            xr = x_ref[n0:n0 + nn, c * 4 * L:(c + 1) * 4 * L]
            if nn < L:
                xr = jnp.concatenate([xr, ones], axis=0)
            pk = jnp.concatenate([_up(pk_ref[4 * c + j]) for j in range(4)], axis=1)
            gp = lax.dot_general(pk, xr, NT, preferred_element_type=F32)
            if c == 0:
                g_ref[nt] = gp
            else:
                g_ref[nt] = g_ref[nt] + gp

    def fold_z():
        lane = lax.broadcasted_iota(jnp.int32, (D, L), 1)
        g3 = g_ref[3]
        zb_ref[...] = jnp.where(lane < 64, pltpu.roll(g3, 64, 1), g3)

    def fold_kv():
        rh = lax.broadcasted_iota(jnp.int32, (GR, GR), 0) // DH
        ch = lax.broadcasted_iota(jnp.int32, (GR, GR), 1) // DH
        same = rh == ch
        kvs = []
        for j in range(4):
            rs = slice(GR * j, GR * (j + 1))
            gb = jnp.concatenate([g_ref[0, rs, :], g_ref[1, rs, :], g_ref[2, rs, :],
                                  g_ref[3, rs, 0:64]], axis=1).astype(BF16)
            kvt = lax.dot_general(_lhs(wvt_ref, GR * j, GR * (j + 1)), gb, NT,
                                  preferred_element_type=F32)
            kvs.append(jnp.where(same, kvt, 0.0).astype(BF16))
        return kvs

    def fold_m(kvs):
        for j in range(4):
            mt = jnp.dot(_up(wo_ref[j, :, 0:GR]), kvs[j], preferred_element_type=F32)
            wo_ref[j, :, 0:GR] = _pk(mt.astype(BF16))

    scale = DH ** -0.5
    lane8 = lax.broadcasted_iota(jnp.int32, (8, L), 1)
    sub8 = lax.broadcasted_iota(jnp.int32, (8, L), 0)
    top = sub8 < 4

    def proj(i):
        res = jnp.dot(_lhs(w2_ref), x_ref[:, i * L:(i + 1) * L],
                      preferred_element_type=F32)
        g = _recip(1.0 + jnp.exp(-res[0:8]))
        q_ref[i] = res[A0:A0 + D]
        k_ref[i] = res[A0 + D:A0 + 2 * D]
        v_ref[i] = res[A0 + 2 * D:A0 + 3 * D]
        omg = 1.0 - g
        for hp in range(H // 2):
            r0 = 56 * hp
            pq = [_phi(res[QB0 + r0 + 8 * j:QB0 + r0 + 8 * j + 8]) for j in range(7)]
            pr = [pq[j] * zb_ref[r0 + 8 * j:r0 + 8 * j + 8, :] for j in range(7)]
            sa = pr[0] + pr[1] + pr[2] + jnp.where(top, pr[3], 0.0)
            sb = pr[4] + pr[5] + pr[6] + jnp.where(top, 0.0, pr[3])
            rs = []
            for s in (sa, sb):
                s = s + pltpu.roll(s, 4, 0)
                s = s + pltpu.roll(s, 2, 0)
                s = s + pltpu.roll(s, 1, 0)
                rs.append(omg * _recip(s + 1e-6))
            rm = jnp.where(top, rs[0], rs[1])
            fac = [rs[0]] * 3 + [rm] + [rs[1]] * 3
            yb = [pq[j] * fac[j] for j in range(7)]
            y0 = _yrow_b(r0) // 2
            if hp % 2 == 0:
                carry = yb[6]
                y_ref[i, y0:y0 + 24, :] = _pk(jnp.concatenate(yb[0:6], axis=0).astype(BF16))
            else:
                y_ref[i, y0 - 4:y0 + 28, :] = _pk(jnp.concatenate([carry] + yb, axis=0).astype(BF16))
        return g

    def delay(cur, prev, sh):
        if sh == 0:
            return cur
        if prev is not None:
            cur = jnp.where(lane8 < L - sh, cur, prev)
        return pltpu.roll(cur, sh, 1)

    def advance(cur, nxt, sh):
        if nxt is not None:
            cur = jnp.where(lane8 >= sh, cur, nxt)
        return pltpu.roll(cur, L - sh, 1)

    his = {}
    ps = {}

    def logits(i, g):
        his[i] = []
        ps[i] = []
        for hh in range(2):
            lo = [None] * 4
            hi = [None] * 4
            for d in range(DH):
                r = H * d + 8 * hh
                q = q_ref[i, r:r + 8, :]
                qa = advance(q, q_ref[i + 1, r:r + 8, :] if i + 1 < NB else None, 8)
                kc = k_ref[i, r:r + 8, :]
                kp = k_ref[i - 1, r:r + 8, :] if i > 0 else None
                for w in range(4):
                    kd = delay(kc, kp, 2 * w)
                    t0 = q * kd
                    t1 = qa * kd
                    lo[w] = t0 if d == 0 else lo[w] + t0
                    hi[w] = t1 if d == 0 else hi[w] + t1
            his[i].append(hi)
            lg = lo + [delay(hi[w], his[i - 1][hh][w] if i > 0 else None, 8) for w in range(4)]
            lg = [l * scale for l in lg]
            if i == 0:
                lg = [jnp.where(lane8 >= 2 * w, lg[w], -1e9) for w in range(W)]
            m = functools.reduce(jnp.maximum, lg)
            p = [jnp.exp(l - m) for l in lg]
            f = g * _recip(functools.reduce(jnp.add, p))
            ps[i].append([pw * f for pw in p])

    def av(i):
        pa = [[advance(ps[i][hh][4 + w], ps[i + 1][hh][4 + w] if i + 1 < NB else None, 8)
               for w in range(4)] for hh in range(2)]
        for d in range(DH):
            o = []
            for hh in range(2):
                r = H * d + 8 * hh
                vc = v_ref[i, r:r + 8, :]
                vp = v_ref[i - 1, r:r + 8, :] if i > 0 else None
                lo = hi = None
                for w in range(4):
                    vd = delay(vc, vp, 2 * w)
                    t0 = ps[i][hh][w] * vd
                    t1 = pa[hh][w] * vd
                    lo = t0 if lo is None else lo + t0
                    hi = t1 if hi is None else hi + t1
                hp_ = oh_ref[i - 1, r:r + 8, :] if i > 0 else jnp.zeros((8, L), F32)
                if i + 1 < NB:
                    oh_ref[i, r:r + 8, :] = hi
                o.append(lo + delay(hi, hp_, 8))
            y0 = _yrow_a(H * d) // 2
            y_ref[i, y0:y0 + 8, :] = _pk(jnp.concatenate(o, axis=0).astype(BF16))

    def ocopy(i):
        sl = slice(i * L, (i + 1) * L)
        return pltpu.make_async_copy(o_ref.at[:, sl], o_hbm.at[:, sl], osems.at[i])

    def outp(i):
        wo = _lhs(wo_ref, ntiles=7, last=L)
        o_ref[:, i * L:(i + 1) * L] = jnp.dot(wo, _up(y_ref[i]), preferred_element_type=F32).astype(BF16)
        ocopy(i).start()

    c_wbk.wait()
    prep1()
    c_x[0].wait()
    for i in range(0, 2):
        p1_proj(i)
    c_x[1].wait()
    for i in range(2, 6):
        p1_proj(i)
    p1_g(0)
    c_x[2].wait()
    for i in range(6, 10):
        p1_proj(i)
    p1_g(1)
    for i in range(10, 12):
        p1_proj(i)
    for c in c_w:
        c.wait()
    prep2()
    for i in range(12, 14):
        p1_proj(i)
    p1_g(2)
    for i in range(14, 16):
        p1_proj(i)
    gs = {}
    kvs = None
    p1_g(3)
    fold_z()
    for step in range(NB + 2):
        if step < NB:
            gs[step] = proj(step)
        if step == 0:
            kvs = fold_kv()
        if step == 1:
            fold_m(kvs)
        if 0 <= step - 1 < NB:
            logits(step - 1, gs[step - 1])
        if 0 <= step - 2 < NB:
            av(step - 2)
        if step in (6, 10, 14, 17):
            c = {6: 0, 10: 1, 14: 2, 17: 3}[step]
            for i in range(4 * c, 4 * c + 4):
                outp(i)
    for i in range(NB):
        ocopy(i).wait()


@jax.jit
def pallas_gated_mix__sliding_local_dilated__linear_attn_block__prompt_kernel(
    A_x, A_wqkv, A_wo, B_x, B_wqkv, B_wo, gate_w,
):
    xt = A_x[0].T
    out = pl.pallas_call(
        _kernel,
        out_shape=jax.ShapeDtypeStruct((D, S), BF16),
        in_specs=[pl.BlockSpec(memory_space=pl.ANY)] * 6,
        out_specs=pl.BlockSpec(memory_space=pl.ANY),
        scratch_shapes=[
            pltpu.VMEM((D, S), BF16),
            pltpu.VMEM((D, 3 * D), BF16),
            pltpu.VMEM((D, D), BF16),
            pltpu.VMEM((D, 3 * D), BF16),
            pltpu.VMEM((D, D), BF16),
            pltpu.VMEM((D,), BF16),
            pltpu.VMEM((D, S), BF16),
            pltpu.VMEM((KT, 4 * D, L), F32),
            pltpu.VMEM((KT, D // 2, L), U32),
            pltpu.VMEM((KT, 8 + 2 * D, L), U32),
            pltpu.VMEM((7, D // 2, L), U32),
            pltpu.VMEM((KT, D // 2, L), U32),
            pltpu.VMEM((NB, D // 2, L), U32),
            pltpu.VMEM((KT, D, L), F32),
            pltpu.VMEM((D, L), F32),
            pltpu.VMEM((NB, D, L), F32),
            pltpu.VMEM((NB, D, L), F32),
            pltpu.VMEM((NB, D, L), F32),
            pltpu.VMEM((NB, D, L), F32),
            pltpu.VMEM((NB, D, L), U32),
            pltpu.SemaphoreType.DMA((10,)),
            pltpu.SemaphoreType.DMA((NB,)),
        ],
        compiler_params=pltpu.CompilerParams(vmem_limit_bytes=64 * 1024 * 1024),
    )(xt, A_wqkv, A_wo, B_wqkv, B_wo, gate_w)
    return out.T[None]
```

```python
import functools
import jax
import jax.numpy as jnp
from jax import lax
import jax.experimental.pallas as pl
import jax.experimental.pallas.tpu as pltpu

S = 2048
D = 448
H = 16
DH = 28
W = 8
L = 128
NB = S // L
NP = NB // 2
KT = 4
GR = 4 * DH
RA = 192
HD = D // 2
K1 = 256
K2 = D - K1
F32 = jnp.float32
BF16 = jnp.bfloat16
U32 = jnp.uint32
NT = (((1,), (1,)), ((), ()))
FP = 6
GO = (1, 3, 5, 7, 2, 4, 6)
G0 = (3, 4, 1, 5, 7, 2, 6)
SV = 1
OO = 0
QV = 1


def _ktile(kt):
    return kt * L, min((kt + 1) * L, D)


def _rows(parts):
    return jnp.concatenate(parts, axis=0)


def _cols(parts):
    return jnp.concatenate(parts, axis=1)


def _dot(a, b):
    return jnp.dot(a, b, preferred_element_type=F32)


def _dot_nt(a, b):
    return lax.dot_general(a, b, NT, preferred_element_type=F32)


def _phi(t):
    return jnp.where(t > 0, t + 1.0, jnp.exp(t)) + 1e-6


def _recip(x):
    r = pl.reciprocal(x, approx=True)
    return r * (2.0 - x * r)


def _sub_allsum(s):
    ax = s.ndim - 2
    s = s + pltpu.roll(s, 4, ax)
    s = s + pltpu.roll(s, 2, ax)
    return s + pltpu.roll(s, 1, ax)


def _lanes(shape):
    return lax.broadcasted_iota(jnp.int32, shape, len(shape) - 1)


def _delay(cur, prev, sh):
    if sh == 0:
        return cur
    if prev is not None:
        cur = jnp.where(_lanes(cur.shape) < L - sh, cur, prev)
    return pltpu.roll(cur, sh, 1)


def _advance(cur, nxt, sh):
    if nxt is not None:
        cur = jnp.where(_lanes(cur.shape) >= sh, cur, nxt)
    return pltpu.roll(cur, L - sh, 1)


def _strassen_lhs(group):
    zero = jnp.zeros((16, K1 - K2), F32)
    cols = [[] for _ in range(7)]
    for g in range(HD // 16):
        top, bot = group(g), group(g + HD // 16)
        a11, a12, a21, a22 = top[:, 0:K1], top[:, K1:D], bot[:, 0:K1], bot[:, K1:D]
        a22p = _cols([a22, zero])
        vals = (a11 + a22p, a21 + a22p, a11, a22, a11[:, 0:K2] + a12, a21 - a11, a12 - a22)
        for c, v in zip(cols, vals):
            c.append(v)
    return [_rows(c).astype(BF16) for c in cols]


def _kernel(x_hbm, wa_hbm, woa_hbm, wb_hbm, wob_hbm, gw_hbm, o_hbm,
            x_ref, wa_ref, woa_ref, wb_ref, wob_ref, gw_ref, o_ref,
            t_ref, xp_ref, sems):
    def cp(src, dst, n):
        return pltpu.make_async_copy(src, dst, sems.at[n])

    def colcp(src, dst, c0, c1, n):
        return cp(src.at[:, c0:c1], dst.at[:, c0:c1], n)

    groups = [
        [colcp(wb_hbm, wb_ref, 640, 896, 0)],
        [colcp(x_hbm, x_ref, 0, 2 * L, 1), cp(gw_hbm, gw_ref, 1)],
        [colcp(wb_hbm, wb_ref, 384, 640, 2), colcp(x_hbm, x_ref, 2 * L, 4 * L, 2)],
        [colcp(x_hbm, x_ref, 4 * L, S, 3)],
        [cp(wa_hbm, wa_ref, 4), colcp(wb_hbm, wb_ref, 0, 384, 4),
         colcp(wb_hbm, wb_ref, 2 * D, 3 * D, 4), cp(woa_hbm, woa_ref, 4), cp(wob_hbm, wob_ref, 4)],
    ]
    for grp in groups:
        for c in grp:
            c.start()

    def wait(n):
        for c in groups[n]:
            c.wait()

    def wbt(c0, c1):
        return _cols([wb_ref[slice(*_ktile(kt)), c0:c1].T for kt in range(KT)])

    E = {}
    gs, xs, xraw = {}, {}, {}

    def xb(i, r0=0, r1=D):
        if i < 4:
            if i not in xraw:
                xp_ref[i] = pltpu.bitcast(x_ref[:, i * L:(i + 1) * L], U32)
                xraw[i] = True
            return pltpu.bitcast(xp_ref[i], BF16)[r0:r1]
        if (i, r0, r1) not in xraw:
            xraw[i, r0, r1] = _rows([xraw[i, g] for g in range(r0 // 16, r1 // 16)]).astype(BF16)
        return xraw[i, r0, r1]

    def prep_xs(p):
        cs = slice(2 * p * L, (2 * p + 2) * L)
        out = [[] for _ in range(5)]
        acc = []

        def load(g):
            b = x_ref[16 * g:16 * g + 16, cs].astype(F32)
            gw = E['gwb'][16 * g:16 * g + 16]
            t = b * _cols([gw, gw])
            acc[:] = [acc[0] + t if acc else t]
            xraw[2 * p, g], xraw[2 * p + 1, g] = b[:, 0:L], b[:, L:2 * L]
            return b[:, 0:L], b[:, L:2 * L]
        for g in range(K1 // 16):
            b11, b12 = load(g)
            out[3].append(b11 + b12)
            if 16 * g < K2:
                b21, b22 = load(K1 // 16 + g)
                out[0].append(b11 + b22)
                out[1].append(b12 - b22)
                out[2].append(b21 - b11)
                out[4].append(b21 + b22)
            else:
                out[0].append(b11)
                out[1].append(b12)
        xs[p] = [_rows(o).astype(BF16) for o in out]
        xb(2 * p), xb(2 * p + 1), xb(2 * p, 0, K1), xb(2 * p + 1, K1, D)
        g2 = _recip(1.0 + jnp.exp(-_sub_allsum(acc[0][0:8] + acc[0][8:16])))
        gs[2 * p], gs[2 * p + 1] = g2[:, 0:L], g2[:, L:2 * L]

    def strassen(jobs, interleave):
        def run(job, first6):
            a, p, sink = job
            r1, r3, r4, r6, r7 = xs[p]
            rhs = (r1, xb(2 * p, 0, K1), r3, r4, xb(2 * p + 1, K1, D), r6, r7)
            m = lambda n: _dot(a[n - 1], rhs[n - 1])
            if first6:
                m6 = m(6)
            m3, m5 = m(3), m(5)
            sink(0, 2 * p + 1, m3 + m5)
            c22 = m6 + m3 if first6 else m3
            yield
            m2, m4 = m(2), m(4)
            sink(1, 2 * p, m2 + m4)
            c11 = m4 - m5
            c22 = c22 - m2
            yield
            m1, m7 = m(1), m(7)
            sink(0, 2 * p, c11 + (m1 + m7))
            c22 = c22 + m1
            yield
            sink(1, 2 * p + 1, c22 if first6 else c22 + m(6))
            yield

        ga, gb = run(jobs[0], False), run(jobs[1], not interleave)
        for g in ([ga, gb] * 4 if interleave else [ga] * 4 + [gb] * 4):
            next(g)

    def headrows(tile, base, n):
        out = []
        for e in range(DH // 2):
            u = t_ref[tile, pl.ds(base + e, H, stride=DH // 2), :][:, 0:n]
            out.append(lax.bitcast_convert_type(lax.shift_left(u, jnp.uint32(16)), F32))
            out.append(lax.bitcast_convert_type(lax.bitwise_and(u, jnp.uint32(0xFFFF0000)), F32))
        return out

    def permuted(base):
        hr = [headrows(kt, base, _ktile(kt)[1] - _ktile(kt)[0]) for kt in range(KT)]
        return [_cols([hr[kt][d] for kt in range(KT)]) for d in range(DH)]

    def prep_weights():
        for kt in range(KT):
            k0, k1 = _ktile(kt)
            t_ref[kt, 0:3 * HD, 0:k1 - k0] = pltpu.bitcast(wa_ref[k0:k1, :].T, U32)
        E['wq'] = _rows(permuted(0)).astype(BF16)
        E['wk'] = _rows(permuted(HD)).astype(BF16)
        wv = permuted(2 * HD)
        E['lv'] = _strassen_lhs(lambda g: wv[g])
        qbt = wbt(0, 512)
        E['lq'] = _strassen_lhs(lambda g: qbt[16 * g:16 * g + 16].astype(F32))
        E['wvt'] = wbt(2 * D, 3 * D)
        for nt in range(KT):
            n0, n1 = _ktile(nt)
            t_ref[nt, 3 * HD:4 * HD, 0:n1 - n0] = pltpu.bitcast(woa_ref[:, n0:n1], U32)
        pa = permuted(3 * HD)
        mixed = []
        for j in range(4):
            mixed += [wob_ref[GR * j:GR * (j + 1), :], pa[j].astype(BF16)]
        E['wo'] = _cols([_rows(mixed).T, _rows(pa[4:]).astype(BF16).T])

    pk, zacc, G = {}, {}, {}

    def pk_sink(i, r0, kb):
        v = _phi(kb)
        for g in range(kb.shape[0] // 32):
            gg = r0 // 32 + g
            pk[i, gg] = v[32 * g:32 * g + 32]
            zacc[gg] = zacc[gg] + pk[i, gg] if gg in zacc else pk[i, gg]

    def pkq(i, half):
        return _rows([pk[i, g] for g in range(half * 7, half * 7 + 7)])

    def kb_chunk(c):
        prep_xs(2 * c)
        prep_xs(2 * c + 1)
        sink = lambda half, i, val: pk_sink(i, half * HD, val)
        strassen([(E['lk'], 2 * c, sink), (E['lk'], 2 * c + 1, sink)], False)

    def g_chunk(c, parts=GO):
        for n in parts:
            for p in (2 * c, 2 * c + 1):
                i, j = 2 * p, 2 * p + 1
                r1, r3, r4, r6, r7 = xs[p]
                xl = (r1, r7, xb(i, 0, K1), xb(j, K1, D), r6, r4, r3)[n - 1]
                pr = (lambda: pkq(i, 0) + pkq(j, 1), lambda: pkq(i, 0), lambda: pkq(i, 1) - pkq(j, 1),
                      lambda: pkq(j, 0) - pkq(i, 0), lambda: pkq(j, 1), lambda: pkq(i, 0) + pkq(i, 1),
                      lambda: pkq(j, 0) + pkq(j, 1))[n - 1]()
                if n % 2:
                    gp = _dot_nt(pr.astype(BF16), xl)
                    G[n] = gp + G[n] if n in G else gp
                else:
                    for u in range(2):
                        gp = _dot_nt(xl, pr[GR * u:GR * (u + 1)].astype(BF16))
                        G[n, u] = gp + G[n, u] if (n, u) in G else gp

    def fold_z():
        z = jnp.sum(_rows([zacc[g] for g in range(D // 32)]), axis=1, keepdims=True)
        E['zb'] = jnp.broadcast_to(z, (D, L))

    def fold_kv():
        ri = lax.broadcasted_iota(jnp.int32, (L, L), 0)
        ci = lax.broadcasted_iota(jnp.int32, (L, L), 1)
        same = jnp.logical_and(ri // DH == ci // DH, ri < GR)
        eye = jnp.where(jnp.logical_and(ri == ci, ri >= GR), 1.0, 0.0)
        E['kvs'] = []
        for j in range(4):
            u = j % 2
            us = slice(GR * u, GR * (u + 1))
            wv = E['wvt'][GR * j:GR * (j + 1)]
            if j < 2:
                ga = (G[1] - G[5] + G[7])[us] + _cols([G[4, u].T, jnp.zeros((GR, K1 - K2), F32)])
                kvt = (_dot_nt(wv[:, 0:K1], ga.astype(BF16))
                       + _dot(wv[:, K1:D], (G[2, u] + G[4, u]).astype(BF16)))
            else:
                gb = (G[1] + G[3])[us, 0:K2] + (G[6, u] - G[2, u]).T
                kvt = _dot_nt(wv, _cols([(G[3] + G[5])[us], gb]).astype(BF16))
            kvt = _rows([_cols([kvt, jnp.zeros((GR, L - GR), F32)]), jnp.zeros((L - GR, L), F32)])
            E['kvs'].append(jnp.where(same, kvt, eye).astype(BF16))

    def fold_m():
        wo = E['wo']
        tiles = [_dot(wo[:, j * L:(j + 1) * L], E['kvs'][j]) for j in range(4)]
        tiles += [wo[:, j * L:(j + 1) * L].astype(F32) for j in range(4, 6)]
        cols = [[] for _ in range(7)]
        for g in range(HD // 16):
            def q(half, odd):
                r0 = half * HD + 16 * g
                return _cols([tiles[2 * t + odd][r0:r0 + 16] for t in range(3)])
            a11, a12, a21, a22 = q(0, 0), q(0, 1), q(1, 0), q(1, 1)
            for c, v in zip(cols, (a11 + a22, a21 + a22, a11, a22, a11 + a12, a21 - a11, a12 - a22)):
                c.append(v)
        E['lo'] = [_rows(c).astype(BF16) for c in cols]
        E['wt'] = (wo[0:HD, 6 * L:7 * L], wo[HD:D, 6 * L:7 * L])

    scale = DH ** -0.5
    qv, kv, vv, his, ps, oh, ya, yb = {}, {}, {}, {}, {}, {}, {}, {}

    def proj_q(i):
        if i < NB:
            qv[i] = _dot(E['wq'], xb(i))

    def proj_k(i):
        if i < NB:
            kv[i] = _dot(E['wk'], xb(i))
            logits(i)

    def v_sink(half, i, val):
        vv[i, half] = val

    def qb_sink(half, i, res):
        pq = _phi(res)
        pr = (pq * E['zb'][half * HD:(half + 1) * HD]).reshape(4, 56, L)
        pr = [pr[:, 8 * j:8 * j + 8] for j in range(7)]
        top = lax.broadcasted_iota(jnp.int32, (4, 8, L), 1) < 4
        sa = pr[0] + pr[1] + pr[2] + jnp.where(top, pr[3], 0.0)
        sb = pr[4] + pr[5] + pr[6] + jnp.where(top, 0.0, pr[3])
        omg = (1.0 - gs[i])[None]
        ra, rb = [omg * _recip(_sub_allsum(s) + 1e-6) for s in (sa, sb)]
        fac = jnp.concatenate([ra] * 3 + [jnp.where(top, ra, rb)] + [rb] * 3, axis=1)
        yb[i, half] = pq * fac.reshape(HD, L)

    def logits(i):
        acc = [None] * W
        for r in (0, HD):
            q = qv[i][r:r + HD]
            qa = _advance(q, qv[i + 1][r:r + HD] if i + 1 < NB else None, 8)
            kc = kv[i][r:r + HD]
            kp = kv[i - 1][r:r + HD] if i > 0 else None
            for w in range(4):
                kd = _delay(kc, kp, 2 * w)
                for u, qq in ((w, q), (w + 4, qa)):
                    t = jnp.sum((qq * kd).reshape(HD // H, H, L), axis=0)
                    acc[u] = t if acc[u] is None else acc[u] + t
        his[i] = acc
        lg = acc[0:4] + [_delay(acc[w], his[i - 1][w] if i > 0 else None, 8) for w in range(4, W)]
        lg = [l * scale for l in lg]
        if i == 0:
            lg = [jnp.where(_lanes((H, L)) >= 2 * w, lg[w], -1e9) for w in range(W)]
        m = functools.reduce(jnp.maximum, lg)
        p = [jnp.exp(l - m) for l in lg]
        f = _rows([gs[i], gs[i]]) * _recip(functools.reduce(jnp.add, p))
        ps[i] = [pw * f for pw in p]

    def av(i):
        pa = ps[i][0:4] + [_advance(ps[i][w], ps[i + 1][w] if i + 1 < NB else None, 8)
                           for w in range(4, W)]
        pa = [_rows([t] * (HD // H)) for t in pa]
        o = []
        for half in range(2):
            lo = hi = None
            for w in range(4):
                vd = _delay(vv[i, half], vv[i - 1, half] if i > 0 else None, 2 * w)
                t0 = pa[w] * vd
                t1 = pa[w + 4] * vd
                lo = t0 if lo is None else lo + t0
                hi = t1 if hi is None else hi + t1
            oh[i, half] = hi
            o.append(lo + _delay(hi, oh[i - 1, half] if i > 0 else jnp.zeros((HD, L), F32), 8))
        ya[i] = _rows(o)

    def ytile(i, t):
        if t < 4:
            return _rows([yb[i, t // 2][GR * (t % 2):GR * (t % 2 + 1)], ya[i][H * t:H * (t + 1)]])
        return ya[i][L * t - D:L * (t + 1) - D]

    def outp(p):
        i, j = 2 * p, 2 * p + 1
        a, wt = E['lo'], E['wt']

        def mm(n, rhs):
            return _dot(a[n - 1], rhs.astype(BF16))

        def put(half, blk, val, n=1):
            sl = slice(blk * L, (blk + 1) * L)
            val = val.astype(BF16)
            for u in range(n):
                r0 = u * HD // n
                rs = slice(half * HD + r0, half * HD + r0 + HD // n)
                o_ref[rs, sl] = val[r0:r0 + HD // n]
                cp(o_ref.at[rs, sl], o_hbm.at[rs, sl], 5).start()

        b11, b21, b12, b22 = [_rows([ytile(blk, 2 * t + odd) for t in range(3)])
                              for blk in (i, j) for odd in range(2)]
        ti, tj = ytile(i, 6).astype(BF16), ytile(j, 6).astype(BF16)
        m3 = mm(3, b12 - b22)
        t12 = _dot(wt[0], tj)
        m5 = mm(5, b22)
        put(0, j, m3 + t12 + m5)
        m4 = mm(4, b21 - b11)
        c11 = m4 - m5
        m2 = mm(2, b11)
        t21 = _dot(wt[1], ti)
        put(1, i, m4 + m2 + t21)
        c22 = m3 - m2
        m1 = mm(1, b11 + b22)
        c11 = c11 + m1
        c22 = c22 + m1
        m7 = mm(7, b21 + b22) + _dot(wt[0], ti)
        put(0, i, c11 + m7)
        m6 = mm(6, b11 + b12) + _dot(wt[1], tj)
        put(1, j, c22 + m6, 2 if p == NP - 1 else 1)

    wait(0)
    w1b = wbt(640, 896)
    wait(1)
    for i in range(0, 2):
        pk_sink(i, RA, _dot(w1b, xb(i)))
    E['gwb'] = jnp.broadcast_to(gw_ref[...].reshape(1, D).astype(F32), (L, D)).T
    prep_xs(0)
    wait(2)
    w1a = wbt(384, 640)[64:256]
    for i in range(2, 4):
        pk_sink(i, RA, _dot(w1b, xb(i)))
    for i in range(0, 4):
        pk_sink(i, 0, _dot(w1a, xb(i)))
    w1 = _rows([w1a, w1b])
    E['lk'] = _strassen_lhs(lambda g: w1[16 * g:16 * g + 16].astype(F32))
    prep_xs(1)
    g_chunk(0, G0[:6])
    wait(3)
    g_chunk(0, G0[6:])
    kb_chunk(1)
    g_chunk(1)
    kb_chunk(2)
    kb_chunk(3)
    wait(4)
    fold_z()
    prep_weights()
    g_chunk(2)
    g_chunk(3)
    proj_q(0)
    proj_q(1)
    proj_k(0)
    for p in range(NP):
        proj_q(2 * p + 2)
        if p == FP:
            fold_kv()
        proj_k(2 * p + 1)
        proj_q(2 * p + 3)
        if p == FP:
            fold_m()
        proj_k(2 * p + 2)
        jq, jv = (E['lq'], p, qb_sink), (E['lv'], p, v_sink)
        strassen([jv, jq] if SV else [jq, jv], True)
    for i in range(NB):
        av(i)
    for p in range(NP):
        outp(p)
    cp(o_ref, o_hbm, 5).wait()


@jax.jit
def pallas_gated_mix__sliding_local_dilated__linear_attn_block__prompt_kernel(
    A_x, A_wqkv, A_wo, B_x, B_wqkv, B_wo, gate_w,
):
    del B_x
    out = pl.pallas_call(
        _kernel,
        out_shape=jax.ShapeDtypeStruct((D, S), BF16),
        in_specs=[pl.BlockSpec(memory_space=pl.ANY)] * 6,
        out_specs=pl.BlockSpec(memory_space=pl.ANY),
        scratch_shapes=[
            pltpu.VMEM((D, S), BF16),
            pltpu.VMEM((D, 3 * D), BF16),
            pltpu.VMEM((D, D), BF16),
            pltpu.VMEM((D, 3 * D), BF16),
            pltpu.VMEM((D, D), BF16),
            pltpu.VMEM((D,), BF16),
            pltpu.VMEM((D, S), BF16),
            pltpu.VMEM((KT, 4 * HD, L), U32),
            pltpu.VMEM((4, HD, L), U32),
            pltpu.SemaphoreType.DMA((6,)),
        ],
        compiler_params=pltpu.CompilerParams(vmem_limit_bytes=64 * 1024 * 1024,
                                             disable_semaphore_checks=True),
    )(A_x[0].T, A_wqkv, A_wo, B_wqkv, B_wo, gate_w)
    return out.T[None]
```

```python
import functools
import jax
import jax.numpy as jnp
from jax import lax
import jax.experimental.pallas as pl
import jax.experimental.pallas.tpu as pltpu

S = 2048
D = 448
H = 16
DH = 28
W = 8
L = 128
NB = S // L
NP = NB // 2
KT = 4
GR = 4 * DH
RA = 192
HD = D // 2
K1 = 256
K2 = D - K1
F32 = jnp.float32
BF16 = jnp.bfloat16
U32 = jnp.uint32
NT = (((1,), (1,)), ((), ()))
FOLD_AT = 5
PRODUCTS = (4, 2, 5, 1, 7, 3, 6)


def _ktile(kt):
    return kt * L, min((kt + 1) * L, D)


def _rows(parts):
    return jnp.concatenate(parts, axis=0)


def _cols(parts):
    return jnp.concatenate(parts, axis=1)


def _dot(a, b):
    return jnp.dot(a, b, preferred_element_type=F32)


def _dot_nt(a, b):
    return lax.dot_general(a, b, NT, preferred_element_type=F32)


def _phi(t):
    return jnp.where(t > 0, t + 1.0, jnp.exp(t)) + 1e-6


def _recip(x):
    r = pl.reciprocal(x, approx=True)
    return r * (2.0 - x * r)


def _sub_allsum(s):
    ax = s.ndim - 2
    s = s + pltpu.roll(s, 4, ax)
    s = s + pltpu.roll(s, 2, ax)
    return s + pltpu.roll(s, 1, ax)


def _lanes(shape):
    return lax.broadcasted_iota(jnp.int32, shape, len(shape) - 1)


def _delay(cur, prev, sh):
    if sh == 0:
        return cur
    if prev is not None:
        cur = jnp.where(_lanes(cur.shape) < L - sh, cur, prev)
    return pltpu.roll(cur, sh, 1)


def _advance(cur, nxt, sh):
    if nxt is not None:
        cur = jnp.where(_lanes(cur.shape) >= sh, cur, nxt)
    return pltpu.roll(cur, L - sh, 1)


_COMB = {(0, 0): {1: 1, 4: 1, 5: -1, 7: 1}, (0, 1): {3: 1, 5: 1},
         (1, 0): {2: 1, 4: 1}, (1, 1): {1: 1, 2: -1, 3: 1, 6: 1}}


class _Quads:
    def __init__(self, sink, extra=0):
        self.acc, self.sink = {}, sink
        self.left = {q: len(t) + extra for q, t in _COMB.items()}

    def add(self, quad, val, sign=1):
        if quad not in self.acc:
            self.acc[quad] = (val, sign)
        else:
            old, osign = self.acc[quad]
            if osign == sign:
                self.acc[quad] = (val + old, sign)
            else:
                self.acc[quad] = (val - old if sign > 0 else old - val, 1)
        self.left[quad] -= 1
        if self.left[quad] == 0:
            self.sink(quad, self.acc[quad][0])

    def product(self, n, val):
        for quad, terms in _COMB.items():
            if n in terms:
                self.add(quad, val, terms[n])


def _strassen_lhs(group, split=1):
    zero = jnp.zeros((16, K1 - K2), F32)
    cols = [[] for _ in range(7)]
    for g in range(HD // 16):
        top, bot = group(g), group(g + HD // 16)
        a11, a12, a21, a22 = top[:, 0:K1], top[:, K1:D], bot[:, 0:K1], bot[:, K1:D]
        a22p = _cols([a22, zero])
        vals = (a11 + a22p, a21 + a22p, a11, a22, a11[:, 0:K2] + a12, a21 - a11, a12 - a22)
        for c, v in zip(cols, vals):
            c.append(v)
    n = HD // 16 // split
    return [[_rows(c[n * u:n * (u + 1)]).astype(BF16) for c in cols] for u in range(split)]


def _kernel(x_hbm, wa_hbm, woa_hbm, wb_hbm, wob_hbm, gw_hbm, o_hbm,
            x_ref, wa_ref, woa_ref, wb_ref, wob_ref, gw_ref, o_ref,
            t_ref, xp_ref, sems):
    def cp(src, dst, n):
        return pltpu.make_async_copy(src, dst, sems.at[n])

    def colcp(src, dst, c0, c1, n):
        return cp(src.at[:, c0:c1], dst.at[:, c0:c1], n)

    groups = [
        [colcp(wb_hbm, wb_ref, 640, 896, 0)],
        [colcp(x_hbm, x_ref, 0, 2 * L, 1), cp(gw_hbm, gw_ref, 1)],
        [colcp(wb_hbm, wb_ref, 384, 640, 2), colcp(x_hbm, x_ref, 2 * L, 4 * L, 2)],
        [colcp(x_hbm, x_ref, 4 * L, S, 3)],
        [cp(wa_hbm, wa_ref, 4), colcp(wb_hbm, wb_ref, 0, 384, 4),
         colcp(wb_hbm, wb_ref, 2 * D, 3 * D, 4), cp(woa_hbm, woa_ref, 4), cp(wob_hbm, wob_ref, 4)],
    ]
    for grp in groups:
        for c in grp:
            c.start()

    def wait(n):
        for c in groups[n]:
            c.wait()

    def wbt(c0, c1):
        return _cols([wb_ref[slice(*_ktile(kt)), c0:c1].T for kt in range(KT)])

    E = {}
    gs, xs, xraw = {}, {}, {}

    def xb(i, r0=0, r1=D):
        if i < 4:
            if i not in xraw:
                xp_ref[i] = pltpu.bitcast(x_ref[:, i * L:(i + 1) * L], U32)
                xraw[i] = True
            return pltpu.bitcast(xp_ref[i], BF16)[r0:r1]
        if (i, r0, r1) not in xraw:
            xraw[i, r0, r1] = _rows([xraw[i, g] for g in range(r0 // 16, r1 // 16)]).astype(BF16)
        return xraw[i, r0, r1]

    def gate_weights():
        E['gwb'] = jnp.broadcast_to(gw_ref[...].reshape(1, D).astype(F32), (L, D)).T

    def prep_xs(p):
        cs = slice(2 * p * L, (2 * p + 2) * L)
        out = [[] for _ in range(5)]
        acc = []

        def load(g):
            b = x_ref[16 * g:16 * g + 16, cs].astype(F32)
            gw = E['gwb'][16 * g:16 * g + 16]
            t = b * _cols([gw, gw])
            acc[:] = [acc[0] + t if acc else t]
            xraw[2 * p, g], xraw[2 * p + 1, g] = b[:, 0:L], b[:, L:2 * L]
            return b[:, 0:L], b[:, L:2 * L]
        for g in range(K1 // 16):
            b11, b12 = load(g)
            out[3].append(b11 + b12)
            if 16 * g < K2:
                b21, b22 = load(K1 // 16 + g)
                out[0].append(b11 + b22)
                out[1].append(b12 - b22)
                out[2].append(b21 - b11)
                out[4].append(b21 + b22)
            else:
                out[0].append(b11)
                out[1].append(b12)
        r1, r3, r4, r6, r7 = [_rows(o).astype(BF16) for o in out]
        xs[p] = (r1, xb(2 * p, 0, K1), r3, r4, xb(2 * p + 1, K1, D), r6, r7)
        for i in (2 * p, 2 * p + 1):
            xb(i)
            for kt in range(KT):
                xb(i, *_ktile(kt))
        g2 = jax.nn.sigmoid(_sub_allsum(acc[0][0:8] + acc[0][8:16]))
        gs[2 * p], gs[2 * p + 1] = g2[:, 0:L], g2[:, L:2 * L]

    def strassen(lhs, p, sink):
        qs = _Quads(lambda q, v: sink(q[0], 2 * p + q[1], v))
        for n in PRODUCTS:
            qs.product(n, _dot(lhs[n - 1], xs[p][n - 1]))

    def permuted(base):
        cache = {}

        def row(d):
            e = d // 2
            if e not in cache:
                u = _cols([t_ref[kt, pl.ds(base + e, H, stride=DH // 2), :][:, 0:_ktile(kt)[1] - kt * L]
                           for kt in range(KT)])
                cache[e] = (lax.shift_left(u, jnp.uint32(16)), lax.bitwise_and(u, jnp.uint32(0xFFFF0000)))
            return lax.bitcast_convert_type(cache[e][d % 2], F32)
        return row

    def prep_weights():
        for kt in range(KT):
            k0, k1 = _ktile(kt)
            t_ref[kt, 0:3 * HD, 0:k1 - k0] = pltpu.bitcast(wa_ref[k0:k1, :].T, U32)
        E['wq'] = _rows(list(map(permuted(0), range(DH)))).astype(BF16)
        E['wk'] = _rows(list(map(permuted(HD), range(DH)))).astype(BF16)
        E['lv'] = _strassen_lhs(permuted(2 * HD), 2)
        E['wqb'] = wbt(0, 384)
        E['wvt'] = wbt(2 * D, 3 * D)
        for nt in range(KT):
            n0, n1 = _ktile(nt)
            t_ref[nt, 3 * HD:4 * HD, 0:n1 - n0] = pltpu.bitcast(woa_ref[:, n0:n1], U32)
        pa = list(map(permuted(3 * HD), range(DH)))
        mixed = []
        for j in range(4):
            mixed += [wob_ref[GR * j:GR * (j + 1), :], pa[j].astype(BF16)]
        E['wo'] = _cols([_rows(mixed).T, _rows(pa[4:]).astype(BF16).T])

    pk, zacc, G = {}, {}, {}

    def pk_sink(i, r0, kb):
        v = _phi(kb)
        for g in range(kb.shape[0] // 32):
            gg = r0 // 32 + g
            pk[i, gg] = v[32 * g:32 * g + 32]
            zacc[gg] = zacc[gg] + pk[i, gg] if gg in zacc else pk[i, gg]

    def pkr(i, r0, r1):
        g0, g1 = r0 // 32, -(-r1 // 32)
        return _rows([pk[i, g] for g in range(g0, g1)])[r0 - 32 * g0:r1 - 32 * g0].astype(BF16)

    def kb_chunk(c):
        for p in (2 * c, 2 * c + 1):
            prep_xs(p)
        for p in (2 * c, 2 * c + 1):
            strassen(E['lk'], p, lambda half, i, val: pk_sink(i, half * HD, val))

    def g_main(blocks, nt, r0=0, r1=D):
        if (r0, r1) == (0, D) and (nt, 0, RA) in G:
            G[nt, 0, D] = _rows([G.pop((nt, 0, RA)), G.pop((nt, RA, D))])
        for i in blocks:
            gp = _dot_nt(pkr(i, r0, r1), xb(i, nt * L, (nt + 1) * L))
            G[nt, r0, r1] = gp + G[nt, r0, r1] if (nt, r0, r1) in G else gp

    def g_tail(blocks):
        for j in range(4):
            for i in blocks:
                gp = _dot_nt(xb(i, 3 * L, D), pkr(i, GR * j, GR * (j + 1)))
                G[j] = gp + G[j] if j in G else gp

    def g_chunk(c):
        for nt in range(3):
            g_main(range(4 * c, 4 * c + 4), nt)
        g_tail(range(4 * c, 4 * c + 4))

    def fold_z():
        z = jnp.sum(_rows([zacc[g] for g in range(D // 32)]), axis=1, keepdims=True)
        E['zb'] = jnp.broadcast_to(z, (D, L))
        E['rz'] = _recip(E['zb'])

    def fold_kv():
        ri = lax.broadcasted_iota(jnp.int32, (L, L), 0)
        ci = lax.broadcasted_iota(jnp.int32, (L, L), 1)
        same = jnp.logical_and(ri // DH == ci // DH, ri < GR)
        eye = jnp.where(jnp.logical_and(ri == ci, ri >= GR), 1.0, 0.0)
        E['kvs'] = []
        for j in range(4):
            rs = slice(GR * j, GR * (j + 1))
            rz = E['rz'][rs]
            gn = _cols([G[nt, 0, D][rs] * rz for nt in range(3)] + [G[j].T * rz[:, 0:64]])
            kvt = _dot_nt(E['wvt'][rs], gn.astype(BF16))
            kvt = _rows([_cols([kvt, jnp.zeros((GR, L - GR), F32)]), jnp.zeros((L - GR, L), F32)])
            E['kvs'].append(jnp.where(same, kvt, eye).astype(BF16))

    def fold_m():
        wo = E['wo']
        tiles = [_dot(wo[:, j * L:(j + 1) * L], E['kvs'][j]) for j in range(4)]
        tiles += [wo[:, j * L:(j + 1) * L].astype(F32) for j in range(4, 6)]
        cols = [[] for _ in range(7)]
        for g in range(HD // 16):
            def q(half, odd):
                r0 = half * HD + 16 * g
                return _cols([tiles[2 * t + odd][r0:r0 + 16] for t in range(3)])
            a11, a12, a21, a22 = q(0, 0), q(0, 1), q(1, 0), q(1, 1)
            for c, v in zip(cols, (a11 + a22, a21 + a22, a11, a22, a11 + a12, a21 - a11, a12 - a22)):
                c.append(v)
        E['lo'] = [_rows(c).astype(BF16) for c in cols]
        E['wt'] = (wo[0:HD, 6 * L:7 * L], wo[HD:D, 6 * L:7 * L])

    scale = DH ** -0.5
    qv, kv, vv, his, ps, oh, ya, yb, qtail = {}, {}, {}, {}, {}, {}, {}, {}, {}

    def proj_q(i):
        if i < NB:
            qv[i] = _dot(E['wq'], xb(i))

    def proj_k(i):
        if i < NB:
            kv[i] = _dot(E['wk'], xb(i))
            logits(i)

    def proj_v(p):
        part = {}
        for u in range(2):
            strassen(E['lv'][u], p, lambda half, i, val: part.setdefault((i, half), []).append(val))
        for key, val in part.items():
            vv[key] = _rows(val)

    def proj_qb(i):
        if i in qtail:
            res = _rows([_dot(E['wqb'], xb(i)), qtail[i]])
        else:
            res = _dot(_rows([E['wqb'], E['wqt']]), xb(i))
        top = lax.broadcasted_iota(jnp.int32, (4, 8, L), 1) < 4
        omg = (1.0 - gs[i])[None]
        for half in range(2):
            rs = slice(half * HD, (half + 1) * HD)
            pz = _phi(res[rs]) * E['zb'][rs]
            pr = pz.reshape(4, 56, L)
            pr = [pr[:, 8 * j:8 * j + 8] for j in range(7)]
            sa = pr[0] + pr[1] + pr[2] + jnp.where(top, pr[3], 0.0)
            sb = pr[4] + pr[5] + pr[6] + jnp.where(top, 0.0, pr[3])
            ra, rb = [omg * _recip(_sub_allsum(s) + 1e-6) for s in (sa, sb)]
            fac = jnp.concatenate([ra] * 3 + [jnp.where(top, ra, rb)] + [rb] * 3, axis=1)
            yb[i, half] = pz * fac.reshape(HD, L)

    def logits(i):
        acc = [None] * W
        for r in (0, HD):
            q = qv[i][r:r + HD]
            qa = _advance(q, qv[i + 1][r:r + HD] if i + 1 < NB else None, 8)
            kc = kv[i][r:r + HD]
            kp = kv[i - 1][r:r + HD] if i > 0 else None
            for w in range(4):
                kd = _delay(kc, kp, 2 * w)
                for u, qq in ((w, q), (w + 4, qa)):
                    t = jnp.sum((qq * kd).reshape(HD // H, H, L), axis=0)
                    acc[u] = t if acc[u] is None else acc[u] + t
        his[i] = acc
        lg = acc[0:4] + [_delay(acc[w], his[i - 1][w] if i > 0 else None, 8) for w in range(4, W)]
        lg = [l * scale for l in lg]
        if i == 0:
            lg = [jnp.where(_lanes((H, L)) >= 2 * w, lg[w], -1e9) for w in range(W)]
        m = functools.reduce(jnp.maximum, lg)
        p = [jnp.exp(l - m) for l in lg]
        f = _rows([gs[i], gs[i]]) * _recip(functools.reduce(jnp.add, p))
        ps[i] = [pw * f for pw in p]

    def av(i):
        pa = ps[i][0:4] + [_advance(ps[i][w], ps[i + 1][w] if i + 1 < NB else None, 8)
                           for w in range(4, W)]
        pa = [_rows([t] * (HD // H)) for t in pa]
        o = []
        for half in range(2):
            lo = hi = None
            for w in range(4):
                vd = _delay(vv[i, half], vv[i - 1, half] if i > 0 else None, 2 * w)
                t0 = pa[w] * vd
                t1 = pa[w + 4] * vd
                lo = t0 if lo is None else lo + t0
                hi = t1 if hi is None else hi + t1
            oh[i, half] = hi
            o.append(lo + _delay(hi, oh[i - 1, half] if i > 0 else jnp.zeros((HD, L), F32), 8))
        ya[i] = _rows(o)

    def ytile(i, t):
        if t < 4:
            return _rows([yb[i, t // 2][GR * (t % 2):GR * (t % 2 + 1)], ya[i][H * t:H * (t + 1)]])
        return ya[i][L * t - D:L * (t + 1) - D]

    def outp(p):
        blks = (2 * p, 2 * p + 1)

        def put(q, val):
            sl = slice(blks[q[1]] * L, (blks[q[1]] + 1) * L)
            val = val.astype(BF16)
            n = 2 if (p == NP - 1 and q == (1, 1)) else 1
            for u in range(n):
                r0 = u * HD // n
                rs = slice(q[0] * HD + r0, q[0] * HD + r0 + HD // n)
                o_ref[rs, sl] = val[r0:r0 + HD // n]
                cp(o_ref.at[rs, sl], o_hbm.at[rs, sl], 5).start()

        b11, b21, b12, b22 = [_rows([ytile(blk, 2 * t + odd) for t in range(3)])
                              for blk in blks for odd in range(2)]
        rhs = (lambda: b11 + b22, lambda: b11, lambda: b12 - b22, lambda: b21 - b11,
               lambda: b22, lambda: b11 + b12, lambda: b21 + b22)
        tail = [ytile(blk, 6).astype(BF16) for blk in blks]
        qs = _Quads(put, extra=1)
        for t in (3, (0, 1), 5, 4, 2, (1, 0), 1, 7, (0, 0), 6, (1, 1)):
            if isinstance(t, tuple):
                qs.add(t, _dot(E['wt'][t[0]], tail[t[1]]))
            else:
                qs.product(t, _dot(E['lo'][t - 1], rhs[t - 1]().astype(BF16)))

    wait(0)
    w1b = wbt(640, 896)
    wait(1)
    for i in range(0, 2):
        pk_sink(i, RA, _dot(w1b, xb(i)))
    gate_weights()
    prep_xs(0)
    for nt in range(2):
        g_main((0, 1), nt, RA, D)
    wait(2)
    w1a = wbt(384, 640)
    E['wqt'] = w1a[0:64]
    for i in range(2, 4):
        pk_sink(i, RA, _dot(w1b, xb(i)))
    for i in range(0, 4):
        res = _dot(w1a, xb(i))
        qtail[i] = res[0:64]
        pk_sink(i, 0, res[64:256])
    w1 = _rows([w1a[64:256], w1b])
    E['lk'] = _strassen_lhs(lambda g: w1[16 * g:16 * g + 16].astype(F32))[0]
    gate_weights()
    prep_xs(1)
    for nt in range(2):
        g_main((2, 3), nt, RA, D)
    for nt in range(2):
        g_main(range(4), nt, 0, RA)
    g_main(range(4), 2)
    wait(3)
    g_tail(range(4))
    for c in range(1, 4):
        kb_chunk(c)
    fold_z()
    g_chunk(1)
    wait(4)
    prep_weights()
    g_chunk(2)
    g_chunk(3)
    proj_q(0)
    proj_q(1)
    proj_k(0)
    for p in range(NP):
        proj_q(2 * p + 2)
        proj_k(2 * p + 1)
        if p == FOLD_AT:
            fold_kv()
        proj_q(2 * p + 3)
        proj_k(2 * p + 2)
        proj_qb(2 * p)
        if p == FOLD_AT:
            fold_m()
        proj_v(p)
        proj_qb(2 * p + 1)
    for i in range(NB):
        av(i)
    for p in range(NP):
        outp(p)
    cp(o_ref, o_hbm, 5).wait()


@jax.jit
def pallas_gated_mix__sliding_local_dilated__linear_attn_block__prompt_kernel(
    A_x, A_wqkv, A_wo, B_x, B_wqkv, B_wo, gate_w,
):
    del B_x
    out = pl.pallas_call(
        _kernel,
        out_shape=jax.ShapeDtypeStruct((D, S), BF16),
        in_specs=[pl.BlockSpec(memory_space=pl.ANY)] * 6,
        out_specs=pl.BlockSpec(memory_space=pl.ANY),
        scratch_shapes=[
            pltpu.VMEM((D, S), BF16),
            pltpu.VMEM((D, 3 * D), BF16),
            pltpu.VMEM((D, D), BF16),
            pltpu.VMEM((D, 3 * D), BF16),
            pltpu.VMEM((D, D), BF16),
            pltpu.VMEM((D,), BF16),
            pltpu.VMEM((D, S), BF16),
            pltpu.VMEM((KT, 4 * HD + 16, L), U32),
            pltpu.VMEM((4, HD, L), U32),
            pltpu.SemaphoreType.DMA((6,)),
        ],
        compiler_params=pltpu.CompilerParams(vmem_limit_bytes=64 * 1024 * 1024,
                                             disable_semaphore_checks=True),
    )(A_x.reshape(S, D).T, A_wqkv, A_wo, B_wqkv, B_wo, gate_w)
    return out.T.reshape(1, S, D)
```

```python
import functools
import jax
import jax.numpy as jnp
from jax import lax
import jax.experimental.pallas as pl
import jax.experimental.pallas.tpu as pltpu

S = 2048
D = 448
H = 16
DH = 28
W = 8
L = 128
NB = S // L
NP = NB // 2
KT = 4
GR = 4 * DH
RA = 192
HD = D // 2
K1 = 256
K2 = D - K1
F32 = jnp.float32
BF16 = jnp.bfloat16
U32 = jnp.uint32
NT = (((1,), (1,)), ((), ()))
FOLD_AT = 6
PRODUCTS = (4, 2, 5, 1, 7, 3, 6)


def _ktile(kt):
    return kt * L, min((kt + 1) * L, D)


def _rows(parts):
    return jnp.concatenate(parts, axis=0)


def _cols(parts):
    return jnp.concatenate(parts, axis=1)


def _dot(a, b):
    return jnp.dot(a, b, preferred_element_type=F32)


def _dot_nt(a, b):
    return lax.dot_general(a, b, NT, preferred_element_type=F32)


def _phi(t):
    return jnp.where(t > 0, t + 1.0, jnp.exp(t)) + 1e-6


def _recip(x):
    r = pl.reciprocal(x, approx=True)
    return r * (2.0 - x * r)


def _rnd(x):
    return x.astype(BF16).astype(F32)


def _rnd_split(x):
    c = x * 65537.0
    return c - (c - x)


def _tree_sum(xs):
    while len(xs) > 1:
        xs = [xs[i] + xs[i + 1] if i + 1 < len(xs) else xs[i] for i in range(0, len(xs), 2)]
    return xs[0]


def _sub_allsum(s):
    ax = s.ndim - 2
    s = s + pltpu.roll(s, 4, ax)
    s = s + pltpu.roll(s, 2, ax)
    return s + pltpu.roll(s, 1, ax)


def _lanes(shape):
    return lax.broadcasted_iota(jnp.int32, shape, len(shape) - 1)


def _delay(cur, prev, sh):
    if sh == 0:
        return cur
    if prev is not None:
        cur = jnp.where(_lanes(cur.shape) < L - sh, cur, prev)
    return pltpu.roll(cur, sh, 1)


def _advance(cur, nxt, sh):
    if nxt is not None:
        cur = jnp.where(_lanes(cur.shape) >= sh, cur, nxt)
    return pltpu.roll(cur, L - sh, 1)


_COMB = {(0, 0): {1: 1, 4: 1, 5: -1, 7: 1}, (0, 1): {3: 1, 5: 1},
         (1, 0): {2: 1, 4: 1}, (1, 1): {1: 1, 2: -1, 3: 1, 6: 1}}


class _Quads:
    def __init__(self, sink, extra=0):
        self.acc, self.sink = {}, sink
        self.left = {q: len(t) + extra for q, t in _COMB.items()}

    def add(self, quad, val, sign=1):
        if quad not in self.acc:
            self.acc[quad] = (val, sign)
        else:
            old, osign = self.acc[quad]
            if osign == sign:
                self.acc[quad] = (val + old, sign)
            else:
                self.acc[quad] = (val - old if sign > 0 else old - val, 1)
        self.left[quad] -= 1
        if self.left[quad] == 0:
            self.sink(quad, self.acc[quad][0])

    def product(self, n, val):
        for quad, terms in _COMB.items():
            if n in terms:
                self.add(quad, val, terms[n])


def _strassen_lhs(group, split=1):
    zero = jnp.zeros((16, K1 - K2), F32)
    cols = [[] for _ in range(7)]
    for g in range(HD // 16):
        top, bot = group(g), group(g + HD // 16)
        a11, a12, a21, a22 = top[:, 0:K1], top[:, K1:D], bot[:, 0:K1], bot[:, K1:D]
        a22p = _cols([a22, zero])
        vals = (a11 + a22p, a21 + a22p, a11, a22, a11[:, 0:K2] + a12, a21 - a11, a12 - a22)
        for c, v in zip(cols, vals):
            c.append(v)
    n = HD // 16 // split
    return [[_rows(c[n * u:n * (u + 1)]).astype(BF16) for c in cols] for u in range(split)]


def _kernel(x_hbm, wa_hbm, woa_hbm, wb_hbm, wob_hbm, gw_hbm, o_hbm,
            x_ref, wa_ref, woa_ref, wb_ref, wob_ref, gw_ref, o_ref,
            t_ref, xp_ref, sems):
    def cp(src, dst, n):
        return pltpu.make_async_copy(src, dst, sems.at[n])

    def colcp(src, dst, c0, c1, n):
        return cp(src.at[:, c0:c1], dst.at[:, c0:c1], n)

    groups = [
        [colcp(wb_hbm, wb_ref, 640, 896, 0)],
        [colcp(x_hbm, x_ref, 0, 2 * L, 1), cp(gw_hbm, gw_ref, 1)],
        [colcp(wb_hbm, wb_ref, 384, 640, 2), colcp(x_hbm, x_ref, 2 * L, 4 * L, 2)],
        [colcp(x_hbm, x_ref, 4 * L, S, 3)],
        [cp(wa_hbm, wa_ref, 4), colcp(wb_hbm, wb_ref, 0, 384, 4),
         colcp(wb_hbm, wb_ref, 2 * D, 3 * D, 4), cp(woa_hbm, woa_ref, 4), cp(wob_hbm, wob_ref, 4)],
    ]
    for grp in groups:
        for c in grp:
            c.start()

    def wait(n):
        for c in groups[n]:
            c.wait()

    def wbt(c0, c1):
        return _cols([wb_ref[slice(*_ktile(kt)), c0:c1].T for kt in range(KT)])

    E = {}
    gs, og, gsum, xs, xraw = {}, {}, {}, {}, {}

    def xb(i, r0=0, r1=D):
        if i < 4:
            if i not in xraw:
                xp_ref[i] = pltpu.bitcast(x_ref[:, i * L:(i + 1) * L], U32)
                xraw[i] = True
            return pltpu.bitcast(xp_ref[i], BF16)[r0:r1]
        if (i, r0, r1) not in xraw:
            xraw[i, r0, r1] = _rows([xraw[i, g] for g in range(r0 // 16, r1 // 16)]).astype(BF16)
        return xraw[i, r0, r1]

    def gate_weights():
        E['gwb'] = jnp.broadcast_to(gw_ref[...].reshape(1, D).astype(F32), (L, D)).T

    def prep_xs(p):
        cs = slice(2 * p * L, (2 * p + 2) * L)
        out = [[] for _ in range(5)]
        acc = []

        def load(g):
            b = x_ref[16 * g:16 * g + 16, cs].astype(F32)
            gw = E['gwb'][16 * g:16 * g + 16]
            acc.append(_rnd(b * _cols([gw, gw])))
            xraw[2 * p, g], xraw[2 * p + 1, g] = b[:, 0:L], b[:, L:2 * L]
            return b[:, 0:L], b[:, L:2 * L]
        for g in range(K1 // 16):
            b11, b12 = load(g)
            out[3].append(b11 + b12)
            if 16 * g < K2:
                b21, b22 = load(K1 // 16 + g)
                out[0].append(b11 + b22)
                out[1].append(b12 - b22)
                out[2].append(b21 - b11)
                out[4].append(b21 + b22)
            else:
                out[0].append(b11)
                out[1].append(b12)
        r1, r3, r4, r6, r7 = [_rows(o).astype(BF16) for o in out]
        xs[p] = (r1, xb(2 * p, 0, K1), r3, r4, xb(2 * p + 1, K1, D), r6, r7)
        for i in (2 * p, 2 * p + 1):
            xb(i)
            for kt in range(KT):
                xb(i, *_ktile(kt))
        u = _tree_sum(acc)
        gsum[p] = u[0:8] + u[8:16]

    def gates():
        u = _rnd(_sub_allsum(_cols([gsum[p] for p in range(NP)])))
        g = _rnd(1.0 / _rnd(1.0 + _rnd(jnp.exp(-u))))
        omg = _rnd(1.0 - g)
        for i in range(NB):
            gs[i], og[i] = g[:, i * L:(i + 1) * L], omg[:, i * L:(i + 1) * L]

    def strassen(lhs, p, sink):
        qs = _Quads(lambda q, v: sink(q[0], 2 * p + q[1], v))
        for n in PRODUCTS:
            qs.product(n, _dot(lhs[n - 1], xs[p][n - 1]))

    def permuted(base):
        cache = {}

        def row(d):
            e = d // 2
            if e not in cache:
                u = _cols([t_ref[kt, pl.ds(base + e, H, stride=DH // 2), :][:, 0:_ktile(kt)[1] - kt * L]
                           for kt in range(KT)])
                cache[e] = (lax.shift_left(u, jnp.uint32(16)), lax.bitwise_and(u, jnp.uint32(0xFFFF0000)))
            return lax.bitcast_convert_type(cache[e][d % 2], F32)
        return row

    def prep_weights():
        for kt in range(KT):
            k0, k1 = _ktile(kt)
            t_ref[kt, 0:3 * HD, 0:k1 - k0] = pltpu.bitcast(wa_ref[k0:k1, :].T, U32)
        E['wq'] = _rows(list(map(permuted(0), range(DH)))).astype(BF16)
        E['wk'] = _rows(list(map(permuted(HD), range(DH)))).astype(BF16)
        E['lv'] = _strassen_lhs(permuted(2 * HD), 2)
        E['wqb'] = wbt(0, 384)
        E['wvt'] = wbt(2 * D, 3 * D)
        for nt in range(KT):
            n0, n1 = _ktile(nt)
            t_ref[nt, 3 * HD:4 * HD, 0:n1 - n0] = pltpu.bitcast(woa_ref[:, n0:n1], U32)
        pa = list(map(permuted(3 * HD), range(DH)))
        mixed = []
        for j in range(4):
            mixed += [wob_ref[GR * j:GR * (j + 1), :], pa[j].astype(BF16)]
        E['wo'] = _cols([_rows(mixed).T, _rows(pa[4:]).astype(BF16).T])

    pk, zacc, G = {}, {}, {}

    def pk_sink(i, r0, kb):
        v = _phi(kb)
        for g in range(kb.shape[0] // 32):
            gg = r0 // 32 + g
            pk[i, gg] = v[32 * g:32 * g + 32]
            zacc[gg] = zacc[gg] + pk[i, gg] if gg in zacc else pk[i, gg]

    def pkr(i, r0, r1):
        g0, g1 = r0 // 32, -(-r1 // 32)
        return _rows([pk[i, g] for g in range(g0, g1)])[r0 - 32 * g0:r1 - 32 * g0].astype(BF16)

    def kb_chunk(c):
        for p in (2 * c, 2 * c + 1):
            prep_xs(p)
        for p in (2 * c, 2 * c + 1):
            strassen(E['lk'], p, lambda half, i, val: pk_sink(i, half * HD, val))

    def g_main(blocks, nt, r0=0, r1=D):
        if (r0, r1) == (0, D) and (nt, 0, RA) in G:
            G[nt, 0, D] = _rows([G.pop((nt, 0, RA)), G.pop((nt, RA, D))])
        for i in blocks:
            gp = _dot_nt(pkr(i, r0, r1), xb(i, nt * L, (nt + 1) * L))
            G[nt, r0, r1] = gp + G[nt, r0, r1] if (nt, r0, r1) in G else gp

    def g_tail(blocks):
        for j in range(4):
            for i in blocks:
                gp = _dot_nt(xb(i, 3 * L, D), pkr(i, GR * j, GR * (j + 1)))
                G[j] = gp + G[j] if j in G else gp

    def g_chunk(c):
        for nt in range(3):
            g_main(range(4 * c, 4 * c + 4), nt)
        g_tail(range(4 * c, 4 * c + 4))

    def fold_z():
        z = jnp.sum(_rows([zacc[g] for g in range(D // 32)]), axis=1, keepdims=True)
        E['zb'] = jnp.broadcast_to(z, (D, L))
        E['rz'] = _recip(E['zb'])

    def fold_kv():
        ri = lax.broadcasted_iota(jnp.int32, (L, L), 0)
        ci = lax.broadcasted_iota(jnp.int32, (L, L), 1)
        same = jnp.logical_and(ri // DH == ci // DH, ri < GR)
        eye = jnp.where(jnp.logical_and(ri == ci, ri >= GR), 1.0, 0.0)
        E['kvs'] = []
        for j in range(4):
            rs = slice(GR * j, GR * (j + 1))
            rz = E['rz'][rs]
            gn = _cols([G[nt, 0, D][rs] * rz for nt in range(3)] + [G[j].T * rz[:, 0:64]])
            kvt = _dot_nt(E['wvt'][rs], gn.astype(BF16))
            kvt = _rows([_cols([kvt, jnp.zeros((GR, L - GR), F32)]), jnp.zeros((L - GR, L), F32)])
            E['kvs'].append(jnp.where(same, kvt, eye).astype(BF16))

    def fold_m():
        wo = E['wo']
        tiles = [_dot(wo[:, j * L:(j + 1) * L], E['kvs'][j]) for j in range(4)]
        tiles += [wo[:, j * L:(j + 1) * L].astype(F32) for j in range(4, 6)]
        cols = [[] for _ in range(7)]
        for g in range(HD // 16):
            def q(half, odd):
                r0 = half * HD + 16 * g
                return _cols([tiles[2 * t + odd][r0:r0 + 16] for t in range(3)])
            a11, a12, a21, a22 = q(0, 0), q(0, 1), q(1, 0), q(1, 1)
            for c, v in zip(cols, (a11 + a22, a21 + a22, a11, a22, a11 + a12, a21 - a11, a12 - a22)):
                c.append(v)
        E['lo'] = [_rows(c).astype(BF16) for c in cols]
        E['wt'] = (wo[0:HD, 6 * L:7 * L], wo[HD:D, 6 * L:7 * L])

    scale = 0.189453125
    qv, kv, vv, his, ps, oh, ya, yb, qtail = {}, {}, {}, {}, {}, {}, {}, {}, {}

    def proj_q(i):
        if i < NB:
            qv[i] = _rnd_split(_dot(E['wq'], xb(i)))

    def proj_k(i):
        if i < NB:
            kv[i] = _rnd_split(_dot(E['wk'], xb(i)))
            logits(i)

    def proj_v(p):
        part = {}
        for u in range(2):
            strassen(E['lv'][u], p, lambda half, i, val: part.setdefault((i, half), []).append(val))
        for key, val in part.items():
            vv[key] = _rows(val)

    def proj_qb(i):
        if i in qtail:
            res = _rows([_dot(E['wqb'], xb(i)), qtail[i]])
        else:
            res = _dot(_rows([E['wqb'], E['wqt']]), xb(i))
        top = lax.broadcasted_iota(jnp.int32, (4, 8, L), 1) < 4
        omg = og[i][None]
        for half in range(2):
            rs = slice(half * HD, (half + 1) * HD)
            pz = _phi(res[rs]) * E['zb'][rs]
            pr = pz.reshape(4, 56, L)
            pr = [pr[:, 8 * j:8 * j + 8] for j in range(7)]
            sa = pr[0] + pr[1] + pr[2] + jnp.where(top, pr[3], 0.0)
            sb = pr[4] + pr[5] + pr[6] + jnp.where(top, 0.0, pr[3])
            ra, rb = [omg * _recip(_sub_allsum(s) + 1e-6) for s in (sa, sb)]
            fac = jnp.concatenate([ra] * 3 + [jnp.where(top, ra, rb)] + [rb] * 3, axis=1)
            yb[i, half] = pz * fac.reshape(HD, L)

    def logits(i):
        acc = [None] * W
        for r in (0, HD):
            q = qv[i][r:r + HD]
            qa = _advance(q, qv[i + 1][r:r + HD] if i + 1 < NB else None, 8)
            kc = kv[i][r:r + HD]
            kp = kv[i - 1][r:r + HD] if i > 0 else None
            for w in range(4):
                kd = _delay(kc, kp, 2 * w)
                for u, qq in ((w, q), (w + 4, qa)):
                    t = jnp.sum((qq * kd).reshape(HD // H, H, L), axis=0)
                    acc[u] = t if acc[u] is None else acc[u] + t
        his[i] = acc
        lg = acc[0:4] + [_delay(acc[w], his[i - 1][w] if i > 0 else None, 8) for w in range(4, W)]
        lg = [_rnd(_rnd_split(l) * scale) for l in lg]
        if i == 0:
            lg = [jnp.where(_lanes((H, L)) >= 2 * w, lg[w], -1e9) for w in range(W)]
        m = functools.reduce(jnp.maximum, lg)
        p = [jnp.exp(l - m) for l in lg]
        f = _rows([gs[i], gs[i]]) * _recip(functools.reduce(jnp.add, p))
        ps[i] = [pw * f for pw in p]

    def av(i):
        pa = ps[i][0:4] + [_advance(ps[i][w], ps[i + 1][w] if i + 1 < NB else None, 8)
                           for w in range(4, W)]
        pa = [_rows([t] * (HD // H)) for t in pa]
        o = []
        for half in range(2):
            lo = hi = None
            for w in range(4):
                vd = _delay(vv[i, half], vv[i - 1, half] if i > 0 else None, 2 * w)
                t0 = pa[w] * vd
                t1 = pa[w + 4] * vd
                lo = t0 if lo is None else lo + t0
                hi = t1 if hi is None else hi + t1
            oh[i, half] = hi
            o.append(lo + _delay(hi, oh[i - 1, half] if i > 0 else jnp.zeros((HD, L), F32), 8))
        ya[i] = _rows(o)

    def ytile(i, t):
        if t < 4:
            return _rows([yb[i, t // 2][GR * (t % 2):GR * (t % 2 + 1)], ya[i][H * t:H * (t + 1)]])
        return ya[i][L * t - D:L * (t + 1) - D]

    def outp(p):
        blks = (2 * p, 2 * p + 1)

        def put(q, val):
            sl = slice(blks[q[1]] * L, (blks[q[1]] + 1) * L)
            val = val.astype(BF16)
            n = 2 if (p == NP - 1 and q == (1, 1)) else 1
            for u in range(n):
                r0 = u * HD // n
                rs = slice(q[0] * HD + r0, q[0] * HD + r0 + HD // n)
                o_ref[rs, sl] = val[r0:r0 + HD // n]
                cp(o_ref.at[rs, sl], o_hbm.at[rs, sl], 5).start()

        b11, b21, b12, b22 = [_rows([ytile(blk, 2 * t + odd) for t in range(3)])
                              for blk in blks for odd in range(2)]
        rhs = (lambda: b11 + b22, lambda: b11, lambda: b12 - b22, lambda: b21 - b11,
               lambda: b22, lambda: b11 + b12, lambda: b21 + b22)
        tail = [ytile(blk, 6).astype(BF16) for blk in blks]
        qs = _Quads(put, extra=1)
        for t in (3, (0, 1), 5, 4, 2, (1, 0), 1, 7, (0, 0), 6, (1, 1)):
            if isinstance(t, tuple):
                qs.add(t, _dot(E['wt'][t[0]], tail[t[1]]))
            else:
                qs.product(t, _dot(E['lo'][t - 1], rhs[t - 1]().astype(BF16)))

    wait(0)
    w1b = wbt(640, 896)
    wait(1)
    for i in range(0, 2):
        pk_sink(i, RA, _dot(w1b, xb(i)))
    gate_weights()
    prep_xs(0)
    for nt in range(2):
        g_main((0, 1), nt, RA, D)
    wait(2)
    w1a = wbt(384, 640)
    E['wqt'] = w1a[0:64]
    for i in range(2, 4):
        pk_sink(i, RA, _dot(w1b, xb(i)))
    for i in range(0, 4):
        res = _dot(w1a, xb(i))
        qtail[i] = res[0:64]
        pk_sink(i, 0, res[64:256])
    w1 = _rows([w1a[64:256], w1b])
    E['lk'] = _strassen_lhs(lambda g: w1[16 * g:16 * g + 16].astype(F32))[0]
    gate_weights()
    prep_xs(1)
    for nt in range(2):
        g_main((2, 3), nt, RA, D)
    for nt in range(2):
        g_main(range(4), nt, 0, RA)
    g_main(range(4), 2)
    wait(3)
    g_tail(range(4))
    for c in range(1, 4):
        kb_chunk(c)
    fold_z()
    gates()
    g_chunk(1)
    wait(4)
    prep_weights()
    g_chunk(2)
    g_chunk(3)
    proj_q(0)
    proj_q(1)
    proj_k(0)
    for p in range(NP):
        proj_q(2 * p + 2)
        proj_k(2 * p + 1)
        if p == FOLD_AT:
            fold_kv()
        proj_q(2 * p + 3)
        proj_k(2 * p + 2)
        proj_qb(2 * p)
        if p == FOLD_AT:
            fold_m()
        proj_v(p)
        proj_qb(2 * p + 1)
    for i in range(NB):
        av(i)
    for p in range(NP):
        outp(p)
    cp(o_ref, o_hbm, 5).wait()


@jax.jit
def pallas_gated_mix__sliding_local_dilated__linear_attn_block__prompt_kernel(
    A_x, A_wqkv, A_wo, B_x, B_wqkv, B_wo, gate_w,
):
    del B_x
    out = pl.pallas_call(
        _kernel,
        out_shape=jax.ShapeDtypeStruct((D, S), BF16),
        in_specs=[pl.BlockSpec(memory_space=pl.ANY)] * 6,
        out_specs=pl.BlockSpec(memory_space=pl.ANY),
        scratch_shapes=[
            pltpu.VMEM((D, S), BF16),
            pltpu.VMEM((D, 3 * D), BF16),
            pltpu.VMEM((D, D), BF16),
            pltpu.VMEM((D, 3 * D), BF16),
            pltpu.VMEM((D, D), BF16),
            pltpu.VMEM((D,), BF16),
            pltpu.VMEM((D, S), BF16),
            pltpu.VMEM((KT, 4 * HD + 16, L), U32),
            pltpu.VMEM((4, HD, L), U32),
            pltpu.SemaphoreType.DMA((6,)),
        ],
        compiler_params=pltpu.CompilerParams(vmem_limit_bytes=64 * 1024 * 1024,
                                             disable_semaphore_checks=True),
    )(A_x.reshape(S, D).T, A_wqkv, A_wo, B_wqkv, B_wo, gate_w)
    return out.T.reshape(1, S, D)
```
